```python
import os as _os
_os.environ.setdefault("JAX_PLATFORMS", "cpu")
import jax
import jax.numpy as jnp

def _softmax(x, axis=-1):
    return jax.nn.softmax(x, axis=axis)
def _gelu(x):
    return jax.nn.gelu(x, approximate=True)
def _silu(x):
    return jax.nn.silu(x)
def _sigmoid(x):
    return jax.nn.sigmoid(x)
def _layernorm(x, axis=-1, eps=1e-5):
    m = jnp.mean(x, axis=axis, keepdims=True)
    v = jnp.var(x, axis=axis, keepdims=True)
    return (x - m) / jnp.sqrt(v + eps)
def _scatter_add(tgt, idx, src, axis=0):
    return tgt.at[idx].add(src)
def _segment_sum(src, seg, n):
    return jax.ops.segment_sum(src, seg, n)
class _Rng:
    def __init__(self, key):
        self._k = key
    def _next(self):
        self._k, sub = jax.random.split(self._k)
        return sub
    def normal(self, shape):
        return jax.random.normal(self._next(), shape, dtype=jnp.bfloat16)
    def randint(self, lo, hi, shape):
        return jax.random.randint(self._next(), shape, lo, hi, dtype=jnp.int32)
    def uniform(self, shape, lo=0.0, hi=1.0):
        return jax.random.uniform(self._next(), shape, jnp.bfloat16, lo, hi)
    def permutation(self, n):
        return jax.random.permutation(self._next(), n)


kernel_name = 'concat_heads__mha_block_cached__mha_block_cached__near_ridge'

def setup_inputs():
    _rng = _Rng(jax.random.key(int.from_bytes(__import__("os").urandom(4), "little")))
    _w = (lambda a: (lambda t: t.astype(jnp.bfloat16) if jnp.issubdtype(t.dtype, jnp.floating) else t)(jnp.asarray(a)))
    def _A_setup():
        B, Sq, D = 32, 32, 640
        H, Sk, Dh = 32, 32, 128
        return {
            "x": _w((lambda *s: _rng.normal(s) * 0.8)(B, Sq, D)),
            "k_cache": _w((lambda *s: _rng.normal(s) * 0.8)(B, H, Sk, Dh)),
            "v_cache": _w((lambda *s: _rng.normal(s) * 0.05)(B, H, Sk, Dh)),
            "wq": _w((lambda *s: _rng.normal(s) * 0.8)(D, H * Dh) * (D ** -0.5)),
            "wo": _w((lambda *s: _rng.normal(s) * 0.05)(H * Dh, D) * ((H * Dh) ** -0.5)),
        }
    _A_in = _A_setup()

    def _B_setup():
        B, Sq, D = 32, 32, 640
        H, Sk, Dh = 32, 32, 128
        return {
            "x": _w((lambda *s: _rng.normal(s) * 0.8)(B, Sq, D)),
            "k_cache": _w((lambda *s: _rng.normal(s) * 0.8)(B, H, Sk, Dh)),
            "v_cache": _w((lambda *s: _rng.normal(s) * 0.05)(B, H, Sk, Dh)),
            "wq": _w((lambda *s: _rng.normal(s) * 0.8)(D, H * Dh) * (D ** -0.5)),
            "wo": _w((lambda *s: _rng.normal(s) * 0.05)(H * Dh, D) * ((H * Dh) ** -0.5)),
        }
    _B_in = _B_setup()

    return {
        "A_x": _A_in["x"],
        "A_k_cache": _A_in["k_cache"],
        "A_v_cache": _A_in["v_cache"],
        "A_wq": _A_in["wq"],
        "A_wo": _A_in["wo"],
        "B_x": _B_in["x"],
        "B_k_cache": _B_in["k_cache"],
        "B_v_cache": _B_in["v_cache"],
        "B_wq": _B_in["wq"],
        "B_wo": _B_in["wo"],
    }

def reference(A_x, A_k_cache, A_v_cache, A_wq, A_wo, B_x, B_k_cache, B_v_cache, B_wq, B_wo):
    def _A_ref(x, k_cache, v_cache, wq, wo):
        B, Sq, D = x.shape
        H, Dh = 32, 128
        q = (lambda x, *d: x.transpose(*d))((x @ wq).reshape(B, Sq, H, Dh), 0, 2, 1, 3)
        scores = jnp.einsum("bhqd,bhkd->bhqk", q, k_cache) * (Dh ** -0.5)
        p = _softmax(scores, axis=-1)
        o = jnp.einsum("bhqk,bhkd->bhqd", p, v_cache)
        return (lambda x, *d: x.transpose(*d))(o, 0, 2, 1, 3).reshape(B, Sq, H * Dh) @ wo

    def _B_ref(x, k_cache, v_cache, wq, wo):
        B, Sq, D = x.shape
        H, Dh = 32, 128
        q = (lambda x, *d: x.transpose(*d))((x @ wq).reshape(B, Sq, H, Dh), 0, 2, 1, 3)
        scores = jnp.einsum("bhqd,bhkd->bhqk", q, k_cache) * (Dh ** -0.5)
        p = _softmax(scores, axis=-1)
        o = jnp.einsum("bhqk,bhkd->bhqd", p, v_cache)
        return (lambda x, *d: x.transpose(*d))(o, 0, 2, 1, 3).reshape(B, Sq, H * Dh) @ wo

    a = _A_ref(A_x, A_k_cache, A_v_cache, A_wq, A_wo)
    b = _B_ref(B_x, B_k_cache, B_v_cache, B_wq, B_wo)
    return jnp.concatenate([a, b], axis=-1)
```

```python
import jax
import jax.numpy as jnp
from jax import lax
from jax.experimental import pallas as pl
from jax.experimental.pallas import tpu as pltpu

B, SQ, D = 32, 32, 640
H, SK, DH = 32, 32, 128
M = B * SQ
SCALE = DH ** -0.5

G = 4
NG = H // G
NS = 2 * NG
CH = 128
NC = M // CH
BPC = CH // SQ
XLO = 256

_STEADY = ("Q0 Q1 D K0 Q2 P0 K1 Q3 P1 O0 K2 Q4 P2 O1 K3 Q5 P3 O2 K4 Q6 P4 O3 "
           "K5 Q7 P5 K6 O4 P6 K7 O5 P7 O6 O7").split()
_FIRST = ("s:wq,xlo,xhi w:wq,xlo s:k,v Q0 Q1 w:xhi s:wo Q2 Q3 Q4 Q5 w:k K0 Q6 K1 Q7 w:v D "
          "K2 K3 P0 P1 w:wo P2 O0 P3 O1 K4 O2 K5 P4 O3 K6 P5 O4 K7 P6 O5 P7 O6 O7").split()


def _softmax_tile(q4, k4):
    st = lax.dot_general(k4, q4, (((1,), (1,)), ((), ())), preferred_element_type=jnp.float32)
    lg = lax.broadcasted_iota(jnp.int32, (SK, G * SQ), 1) // SQ
    c = jnp.where(lg == 0, st[0:32], jnp.where(lg == 1, st[32:64], jnp.where(lg == 2, st[64:96], st[96:128])))
    c = c * SCALE
    e = jnp.exp(c - jnp.max(c, axis=0, keepdims=True))
    p = e / jnp.sum(e, axis=0, keepdims=True)
    return jnp.concatenate([jnp.where(lg == h, p, 0.0) for h in range(G)], axis=0).astype(jnp.bfloat16)


def _pv_tile(pt, v4):
    return lax.dot_general(pt, v4, (((0,), (0,)), ((), ())), preferred_element_type=jnp.float32)


def _kernel(ax, ak, av, awq, awo, bx, bk, bv, bwq, bwo, out,
            x_buf, wq_buf, wo_buf, k_buf, v_buf, q_buf, o_buf, acc, out_buf, sems, xsems, osems):
    def copies(src, g, slot):
        xk, xv, xwq, xwo = src
        return dict(
            wq=pltpu.make_async_copy(xwq.at[:, pl.ds(g * G * DH, G * DH)], wq_buf.at[slot], sems.at[0, slot]),
            k=pltpu.make_async_copy(xk.at[:, pl.ds(g * G * SK, G * SK), :], k_buf.at[slot], sems.at[1, slot]),
            v=pltpu.make_async_copy(xv.at[:, pl.ds(g * G * SK, G * SK), :], v_buf.at[slot], sems.at[2, slot]),
            wo=pltpu.make_async_copy(xwo.at[pl.ds(g * G * DH, G * DH), :], wo_buf.at[slot], sems.at[3, slot]),
        )

    src_a = (ak, av, awq, awo)
    src_b = (bk, bv, bwq, bwo)
    xa_lo = pltpu.make_async_copy(ax.at[pl.ds(0, XLO)], x_buf.at[0, pl.ds(0, XLO)], xsems.at[0])
    xa_hi = pltpu.make_async_copy(ax.at[pl.ds(XLO, M - XLO)], x_buf.at[0, pl.ds(XLO, M - XLO)], xsems.at[1])
    xb = pltpu.make_async_copy(bx, x_buf.at[1], xsems.at[2])

    def step(s, is_first):
        if is_first:
            slot, nxt, br, g, g1 = 0, 1, 0, 0, 1
        else:
            slot = jnp.bitwise_and(s, 1)
            nxt = 1 - slot
            br = jnp.right_shift(s, 3)
            g = jnp.bitwise_and(s, NG - 1)
            g1 = jnp.bitwise_and(s + 1, NG - 1)
        cur = copies(src_a, 0, slot)
        cur["xlo"] = xa_lo
        cur["xhi"] = xa_hi
        probs = {}

        def rows(c):
            return pl.ds(c * CH, CH)

        def q_proj(c):
            q = jnp.dot(x_buf[br, rows(c), :], wq_buf[slot], preferred_element_type=jnp.float32)
            q_buf[rows(c), :] = q.astype(jnp.bfloat16)

        def scores(c):
            for b in range(c * BPC, (c + 1) * BPC):
                r = pl.ds(b * SQ, SQ)
                q4 = jnp.concatenate([q_buf[r, h * DH:(h + 1) * DH] for h in range(G)], axis=0)
                probs[b] = _softmax_tile(q4, k_buf[slot, b])

        def values(c):
            for b in range(c * BPC, (c + 1) * BPC):
                r = pl.ds(b * SQ, SQ)
                o4 = _pv_tile(probs.pop(b), v_buf[slot, b]).astype(jnp.bfloat16)
                for h in range(G):
                    o_buf[r, h * DH:(h + 1) * DH] = o4[h * SQ:(h + 1) * SQ]

        def o_proj(c):
            y = jnp.dot(o_buf[rows(c), :], wo_buf[slot], preferred_element_type=jnp.float32)
            if is_first:
                acc[rows(c), :] = y
                return
            t = jnp.where(g == 0, 0.0, acc[rows(c), :]) + y
            acc[rows(c), :] = t
            out_buf[br, rows(c), :] = t.astype(jnp.bfloat16)

            @pl.when(g == NG - 1)
            def _():
                pltpu.make_async_copy(out_buf.at[br, rows(c)], out.at[rows(c), pl.ds(br * D, D)],
                                      osems.at[br]).start()

        def prefetch():
            if is_first:
                for cp in copies(src_a, 1, 1).values():
                    cp.start()
                return

            @pl.when(s + 1 < NG)
            def _():
                for cp in copies(src_a, g1, nxt).values():
                    cp.start()

            @pl.when(jnp.logical_and(s + 1 >= NG, s + 1 < NS))
            def _():
                for cp in copies(src_b, g1, nxt).values():
                    cp.start()

            @pl.when(s == 2)
            def _():
                xb.start()

        if not is_first:
            for n in ("wq", "k", "v", "wo"):
                cur[n].wait()

            @pl.when(s == NG - 1)
            def _():
                xb.wait()

        stages = {"Q": q_proj, "K": scores, "P": values, "O": o_proj}
        for st in (_FIRST if is_first else _STEADY):
            if st == "D":
                prefetch()
            elif st.startswith("s:"):
                for n in st[2:].split(","):
                    cur[n].start()
            elif st.startswith("w:"):
                for n in st[2:].split(","):
                    cur[n].wait()
            else:
                stages[st[0]](int(st[1:]))

    step(0, True)

    def body(s, carry):
        step(s, False)
        return carry

    lax.fori_loop(1, NS, body, 0)
    for br in range(2):
        pltpu.make_async_copy(out_buf.at[br], out.at[:, pl.ds(br * D, D)], osems.at[br]).wait()


@jax.jit
def pallas_concat_heads__mha_block_cached__mha_block_cached__near_ridge_kernel(
    A_x: jax.Array,
    A_k_cache: jax.Array,
    A_v_cache: jax.Array,
    A_wq: jax.Array,
    A_wo: jax.Array,
    B_x: jax.Array,
    B_k_cache: jax.Array,
    B_v_cache: jax.Array,
    B_wq: jax.Array,
    B_wo: jax.Array,
):
    r3 = lambda t: t.reshape(B, H * SK, DH)
    r2 = lambda t: t.reshape(M, D)
    any_spec = pl.BlockSpec(memory_space=pl.ANY)
    out = pl.pallas_call(
        _kernel,
        out_shape=jax.ShapeDtypeStruct((M, 2 * D), jnp.bfloat16),
        in_specs=[any_spec] * 10,
        out_specs=any_spec,
        scratch_shapes=[
            pltpu.VMEM((2, M, D), jnp.bfloat16),
            pltpu.VMEM((2, D, G * DH), jnp.bfloat16),
            pltpu.VMEM((2, G * DH, D), jnp.bfloat16),
            pltpu.VMEM((2, B, G * SK, DH), jnp.bfloat16),
            pltpu.VMEM((2, B, G * SK, DH), jnp.bfloat16),
            pltpu.VMEM((M, G * DH), jnp.bfloat16),
            pltpu.VMEM((M, G * DH), jnp.bfloat16),
            pltpu.VMEM((M, D), jnp.float32),
            pltpu.VMEM((2, M, D), jnp.bfloat16),
            pltpu.SemaphoreType.DMA((4, 2)),
            pltpu.SemaphoreType.DMA((3,)),
            pltpu.SemaphoreType.DMA((2,)),
        ],
        compiler_params=pltpu.CompilerParams(
            vmem_limit_bytes=64 * 1024 * 1024,
            disable_bounds_checks=True,
        ),
    )(r2(A_x), r3(A_k_cache), r3(A_v_cache), A_wq, A_wo,
      r2(B_x), r3(B_k_cache), r3(B_v_cache), B_wq, B_wo)
    return out.reshape(B, SQ, 2 * D)
```

```python
import jax
import jax.numpy as jnp
from jax import lax
from jax.experimental import pallas as pl
from jax.experimental.pallas import tpu as pltpu

B, SQ, D = 32, 32, 640
H, SK, DH = 32, 32, 128
M = B * SQ
SCALE = DH ** -0.5

G = 4
NG = H // G
NS = 2 * NG
CH = 128
BPC = CH // SQ
NB = 4
XS = (0, 128, 512, M)
KVS = 16
OSPLIT = 384
S_A = 2
S_B = 4

_SEM_X = 4 * NB
_SEM_XB = _SEM_X + len(XS) - 1
_SEM_OUT = _SEM_XB + 1
_SEM_KV = _SEM_OUT + 2
_NSEM = _SEM_KV + 4

_FIRST = ("s:wq,x0,x1,x2,wo,klo,vlo,khi,vhi D w:wq,x0 Q0 w:x1 Q1 Q2 Q3 w:x2 Q4 Q5 Q6 Q7 "
          "w:wo,klo,vlo K0 K1 K2 K3 P0 P1 P2 P3 O0 O1 w:khi,vhi K4 K5 O2 P4 P5 K6 K7 O3 P6 P7 "
          "O4 O5 O6 O7").split()
_SECOND = ("w:wq,k,v Q0 Q1 D K0 Q2 P0 K1 Q3 P1 w:wo O0 K2 Q4 P2 O1 K3 Q5 P3 O2 K4 Q6 P4 O3 "
           "K5 Q7 P5 K6 O4 P6 K7 O5 P7 O6 O7").split()
_BODY = ("Q0 Q1 D K0 Q2 P0 K1 Q3 P1 O0 K2 Q4 P2 O1 K3 Q5 P3 O2 K4 Q6 P4 O3 "
         "K5 Q7 P5 K6 O4 P6 K7 O5 P7 O6 O7").split()
_BODY_LAST = [t for t in _BODY[:-1] if t != "D"] + ["L7", "R7"]


def _softmax_tile(q4, k4):
    st = lax.dot_general(k4, q4, (((1,), (1,)), ((), ())), preferred_element_type=jnp.float32)
    lg = lax.broadcasted_iota(jnp.int32, (SK, G * SQ), 1) // SQ
    c = jnp.where(lg == 0, st[0:32],
                  jnp.where(lg == 1, st[32:64], jnp.where(lg == 2, st[64:96], st[96:128])))
    c = c * SCALE
    e = jnp.exp(c - jnp.max(c, axis=0, keepdims=True))
    p = e / jnp.sum(e, axis=0, keepdims=True)
    return jnp.concatenate([jnp.where(lg == h, p, 0.0) for h in range(G)], axis=0).astype(jnp.bfloat16)


def _pv_tile(pt, v4):
    return lax.dot_general(pt, v4, (((0,), (0,)), ((), ())), preferred_element_type=jnp.float32)


def _kernel(ax, ak, av, awq, awo, bx, bk, bv, bwq, bwo, out,
            x_buf, wq_buf, wo_buf, k_buf, v_buf, q_buf, o_buf, acc, out_buf, sems):
    src_a = (ak, av, awq, awo)
    src_b = (bk, bv, bwq, bwo)

    def copies(src, g, slot):
        xk, xv, xwq, xwo = src
        return dict(
            wq=pltpu.make_async_copy(xwq.at[:, pl.ds(g * G * DH, G * DH)], wq_buf.at[slot], sems.at[slot * 4]),
            k=pltpu.make_async_copy(xk.at[:, pl.ds(g * G * SK, G * SK), :], k_buf.at[slot], sems.at[slot * 4 + 1]),
            v=pltpu.make_async_copy(xv.at[:, pl.ds(g * G * SK, G * SK), :], v_buf.at[slot], sems.at[slot * 4 + 2]),
            wo=pltpu.make_async_copy(xwo.at[pl.ds(g * G * DH, G * DH), :], wo_buf.at[slot], sems.at[slot * 4 + 3]),
        )

    def start_step(s):
        if isinstance(s, int):
            for cp in copies(src_a if s < NG else src_b, s % NG, s % NB).values():
                cp.start()
            return
        g, slot = jnp.bitwise_and(s, NG - 1), jnp.bitwise_and(s, NB - 1)

        @pl.when(s < NG)
        def _():
            for cp in copies(src_a, g, slot).values():
                cp.start()

        @pl.when(jnp.logical_and(s >= NG, s < NS))
        def _():
            for cp in copies(src_b, g, slot).values():
                cp.start()

    def wait_step(slot):
        for cp in copies(src_a, 0, slot).values():
            cp.wait()

    def x_b_copy():
        return pltpu.make_async_copy(bx, x_buf.at[1], sems.at[_SEM_XB])

    def rows(c):
        return pl.ds(c * CH, CH)

    def stages(slot, br, g, mode):
        probs = {}

        def q_proj(c):
            q = jnp.dot(x_buf[br, rows(c), :], wq_buf[slot], preferred_element_type=jnp.float32)
            q_buf[rows(c), :] = q.astype(jnp.bfloat16)

        def scores(c):
            for b in range(c * BPC, (c + 1) * BPC):
                r = pl.ds(b * SQ, SQ)
                q4 = jnp.concatenate([q_buf[r, h * DH:(h + 1) * DH] for h in range(G)], axis=0)
                probs[b] = _softmax_tile(q4, k_buf[slot, b])

        def values(c):
            for b in range(c * BPC, (c + 1) * BPC):
                r = pl.ds(b * SQ, SQ)
                o4 = _pv_tile(probs.pop(b), v_buf[slot, b]).astype(jnp.bfloat16)
                for h in range(G):
                    o_buf[r, h * DH:(h + 1) * DH] = o4[h * SQ:(h + 1) * SQ]

        def o_proj(c, lo=0, hi=D):
            cols = pl.ds(lo, hi - lo)
            y = jnp.dot(o_buf[rows(c), :], wo_buf[slot, :, cols], preferred_element_type=jnp.float32)
            if mode == "init":
                acc[rows(c), cols] = y
                return
            a = acc[rows(c), cols]
            if mode == "maybe_init":
                a = jnp.where(g == 0, 0.0, a)
            t = a + y
            acc[rows(c), cols] = t
            if mode == "maybe_final":
                out_buf[br, rows(c), cols] = t.astype(jnp.bfloat16)

                @pl.when(g == NG - 1)
                def _():
                    pltpu.make_async_copy(out_buf.at[br, rows(c), cols],
                                          out.at[rows(c), pl.ds(br * D + lo, hi - lo)],
                                          sems.at[_SEM_OUT + br]).start()

        return {"Q": q_proj, "K": scores, "P": values, "O": o_proj,
                "L": lambda c: o_proj(c, 0, OSPLIT), "R": lambda c: o_proj(c, OSPLIT, D)}

    def run(schedule, stage, dmas=None, prefetch=None):
        for t in schedule:
            if t == "D":
                prefetch()
            elif t.startswith("s:"):
                for n in t[2:].split(","):
                    dmas[n].start()
            elif t.startswith("w:"):
                for n in t[2:].split(","):
                    dmas[n].wait()
            else:
                stage[t[0]](int(t[1:]))

    dmas = copies(src_a, 0, 0)
    for i in range(len(XS) - 1):
        r = pl.ds(XS[i], XS[i + 1] - XS[i])
        dmas[f"x{i}"] = pltpu.make_async_copy(ax.at[r], x_buf.at[0, r], sems.at[_SEM_X + i])
    for i, (nm, src, buf) in enumerate((("k", ak, k_buf), ("v", av, v_buf))):
        for j, (hn, b0, nb) in enumerate((("lo", 0, KVS), ("hi", KVS, B - KVS))):
            dmas[nm + hn] = pltpu.make_async_copy(src.at[pl.ds(b0, nb), pl.ds(0, G * SK), :],
                                                  buf.at[0, pl.ds(b0, nb)], sems.at[_SEM_KV + 2 * i + j])

    def prefetch_1_2():
        start_step(1)
        start_step(2)

    run(_FIRST, stages(0, 0, 0, "init"), dmas, prefetch_1_2)

    run(_SECOND, stages(1, 0, 1, "mid"), copies(src_a, 1, 1), lambda: start_step(3))

    def body_a(s, carry):
        slot = jnp.bitwise_and(s, NB - 1)
        wait_step(slot)

        def prefetch():
            start_step(s + 2)

            @pl.when(s == S_A)
            def _():
                x_b_copy().start()

        run(_BODY, stages(slot, 0, None, "mid"), prefetch=prefetch)
        return carry

    lax.fori_loop(S_A, S_B, body_a, 0)

    def body_b(it, carry):
        s = S_B + 2 * it
        br = jnp.right_shift(s, 3)
        g = jnp.bitwise_and(s, NG - 1)
        slot0, slot1 = jnp.bitwise_and(s, NB - 1), jnp.bitwise_and(s + 1, NB - 1)
        wait_step(slot0)
        wait_step(slot1)

        @pl.when(s == NG)
        def _():
            x_b_copy().wait()

        def prefetch():
            start_step(s + 2)
            start_step(s + 3)

        run(_BODY, stages(slot0, br, g, "maybe_init"), prefetch=prefetch)
        run(_BODY_LAST, stages(slot1, br, g + 1, "maybe_final"))
        return carry

    lax.fori_loop(0, (NS - S_B) // 2, body_b, 0)

    for br in range(2):
        pltpu.make_async_copy(out_buf.at[br], out.at[:, pl.ds(br * D, D)], sems.at[_SEM_OUT + br]).wait()


@jax.jit
def pallas_concat_heads__mha_block_cached__mha_block_cached__near_ridge_kernel(
    A_x: jax.Array,
    A_k_cache: jax.Array,
    A_v_cache: jax.Array,
    A_wq: jax.Array,
    A_wo: jax.Array,
    B_x: jax.Array,
    B_k_cache: jax.Array,
    B_v_cache: jax.Array,
    B_wq: jax.Array,
    B_wo: jax.Array,
):
    r3 = lambda t: t.reshape(B, H * SK, DH)
    r2 = lambda t: t.reshape(M, D)
    any_spec = pl.BlockSpec(memory_space=pl.ANY)
    out = pl.pallas_call(
        _kernel,
        out_shape=jax.ShapeDtypeStruct((M, 2 * D), jnp.bfloat16),
        in_specs=[any_spec] * 10,
        out_specs=any_spec,
        scratch_shapes=[
            pltpu.VMEM((2, M, D), jnp.bfloat16),
            pltpu.VMEM((NB, D, G * DH), jnp.bfloat16),
            pltpu.VMEM((NB, G * DH, D), jnp.bfloat16),
            pltpu.VMEM((NB, B, G * SK, DH), jnp.bfloat16),
            pltpu.VMEM((NB, B, G * SK, DH), jnp.bfloat16),
            pltpu.VMEM((M, G * DH), jnp.bfloat16),
            pltpu.VMEM((M, G * DH), jnp.bfloat16),
            pltpu.VMEM((M, D), jnp.float32),
            pltpu.VMEM((2, M, D), jnp.bfloat16),
            pltpu.SemaphoreType.DMA((_NSEM,)),
        ],
        compiler_params=pltpu.CompilerParams(
            vmem_limit_bytes=64 * 1024 * 1024,
            disable_bounds_checks=True,
        ),
    )(r2(A_x), r3(A_k_cache), r3(A_v_cache), A_wq, A_wo,
      r2(B_x), r3(B_k_cache), r3(B_v_cache), B_wq, B_wo)
    return out.reshape(B, SQ, 2 * D)
```

```python
import math

import jax
import jax.numpy as jnp
from jax import lax
from jax.experimental import pallas as pl
from jax.experimental.pallas import tpu as pltpu

B, SQ, D = 32, 32, 640
H, SK, DH = 32, 32, 128
M = B * SQ
SCALE_LOG2E = DH ** -0.5 * math.log2(math.e)

G = 4
NG = H // G
CH = 128
BPC = CH // SQ
NB = 4
NIT = 2 * NG // NB
XS = (0, 128, 256, 512, 896, M)
KBS = (0, 16, B)
VBS = (0, 8, 16, B)
OSPLIT = 384

_SLOT0 = "wq x0 x1 x2 x3 x4 k0 v0 v1 woL woR k1 v2 po0 po1 pq0 pq1".split()
_SLOTN = ("wq", "k", "v", "wo")
_SEM = {(0, n): i for i, n in enumerate(_SLOT0)}
_SEM.update({(j, n): len(_SLOT0) + 4 * (j - 1) + i for j in range(1, NB) for i, n in enumerate(_SLOTN)})
_SEM_OUT = len(_SEM)

_TAIL = "K2 Q4 P2 O1 K3 Q5 P3 O2 K4 Q6 P4 O3 K5 Q7 P5 K6 O4 P6 K7 O5 P7 O6"
_SCHED = (
    "w:wq,x0 Q0 w:x1 Q1 D w:x2 Q2 Q3 w:x3 Q4 Q5 Q6 w:x4 Q7 w:k0,v0 K0 K1 K2 K3 P0 P1 w:v1 P2 P3 "
    "w:woL L0 w:woR R0 O1 w:k1 K4 K5 O2 w:po0,v2 P4 P5 K6 K7 O3 P6 P7 O4 O5 O6 O7",
    "w:po1,wq Q0 Q1 D w:k K0 Q2 w:pq0,v P0 K1 Q3 P1 w:pq1,wo O0 " + _TAIL + " O7",
    "w:wq Q0 Q1 D w:k K0 Q2 w:v P0 K1 Q3 P1 w:wo O0 " + _TAIL + " O7",
    "w:wq Q0 Q1 D w:k K0 Q2 w:v P0 K1 Q3 P1 w:wo O0 " + _TAIL + " L7 R7",
)


def _interleave(tokens):
    out, i = [], 0
    while i < len(tokens):
        j = i + 1
        while j < len(tokens) and tokens[j][0] not in "QKPOLR":
            j += 1
        if tokens[i][0] == "K" and j < len(tokens) and tokens[j][0] == "Q":
            c, d = int(tokens[i][1:]), int(tokens[j][1:])
            for u in range(2):
                out += [f"k{4 * c + 2 * u + w}" for w in range(2)] + [f"q{4 * d + 2 * u + w}" for w in range(2)]
            out += tokens[i + 1:j]
            i = j + 1
        else:
            out.append(tokens[i])
            i += 1
    return out


_SCHED = tuple(_interleave(s.split()) for s in _SCHED)


def _softmax_tile(q4, k4):
    st = lax.dot_general(k4, q4, (((1,), (1,)), ((), ())), preferred_element_type=jnp.float32)
    lg = lax.broadcasted_iota(jnp.int32, (SK, G * SQ), 1) // SQ
    c = jnp.where(lg == 0, st[0:32],
                  jnp.where(lg == 1, st[32:64], jnp.where(lg == 2, st[64:96], st[96:128])))
    e = jnp.exp2((c - jnp.max(c, axis=0, keepdims=True)) * SCALE_LOG2E)
    p = e / jnp.sum(e, axis=0, keepdims=True)
    return jnp.concatenate([jnp.where(lg == h, p, 0.0) for h in range(G)], axis=0).astype(jnp.bfloat16)


def _kernel(ax, ak, av, awq, awo, bx, bk, bv, bwq, bwo, out,
            x_buf, wq_buf, wo_buf, k_buf, v_buf, q_buf, o_buf, acc, out_buf, sems):
    srcs = ((ax, ak, av, awq, awo), (bx, bk, bv, bwq, bwo))

    def copy(j, n, br=0, g=0):
        xs, xk, xv, xwq, xwo = srcs[br]
        sem = sems.at[_SEM[(0 if n[0] in "xp" else j, n)]]
        hs, gs = pl.ds(g * G * SK, G * SK), pl.ds(g * G * DH, G * DH)
        if n == "wq":
            return pltpu.make_async_copy(xwq.at[:, gs], wq_buf.at[j], sem)
        if n == "wo":
            return pltpu.make_async_copy(xwo.at[gs, :], wo_buf.at[j], sem)
        if n in ("woL", "woR"):
            cols = pl.ds(0, OSPLIT) if n == "woL" else pl.ds(OSPLIT, D - OSPLIT)
            return pltpu.make_async_copy(xwo.at[gs, cols], wo_buf.at[j, :, cols], sem)
        if n in ("k", "v"):
            src, buf = (xk, k_buf) if n == "k" else (xv, v_buf)
            return pltpu.make_async_copy(src.at[:, hs, :], buf.at[j], sem)
        if n[0] == "p":
            buf = wo_buf if n[1] == "o" else wq_buf
            return pltpu.make_async_copy(xwq.at[pl.ds(0, 16), pl.ds(0, 128)],
                                         buf.at[NB, pl.ds(16 * int(n[2]), 16), pl.ds(0, 128)], sem)
        i = int(n[1:])
        if n[0] == "x":
            r = pl.ds(XS[i], XS[i + 1] - XS[i])
            return pltpu.make_async_copy(xs.at[r], x_buf.at[br, r], sem)
        bs, src, buf = (KBS, xk, k_buf) if n[0] == "k" else (VBS, xv, v_buf)
        r = pl.ds(bs[i], bs[i + 1] - bs[i])
        return pltpu.make_async_copy(src.at[r, hs, :], buf.at[j, r], sem)

    def start_slot(j, br, g, with_x=False):
        for n in (_SLOT0 if j == 0 else _SLOTN):
            if with_x or n[0] != "x":
                copy(j, n, br, g).start()

    def rows(c):
        return pl.ds(c * CH, CH)

    def stages(slot, br, g):
        probs = {}

        def q_head(c, cols):
            q = jnp.dot(x_buf[br, rows(c), :], wq_buf[slot, :, cols], preferred_element_type=jnp.float32)
            q_buf[rows(c), cols] = q.astype(jnp.bfloat16)

        def score(b):
            r = pl.ds(b * SQ, SQ)
            q4 = jnp.concatenate([q_buf[r, h * DH:(h + 1) * DH] for h in range(G)], axis=0)
            probs[b] = _softmax_tile(q4, k_buf[slot, b])

        def value(b):
            r = pl.ds(b * SQ, SQ)
            o4 = lax.dot_general(probs.pop(b), v_buf[slot, b], (((0,), (0,)), ((), ())),
                                 preferred_element_type=jnp.float32).astype(jnp.bfloat16)
            for h in range(G):
                o_buf[r, h * DH:(h + 1) * DH] = o4[h * SQ:(h + 1) * SQ]

        def o_proj(c, lo=0, hi=D):
            cols = pl.ds(lo, hi - lo)
            y = jnp.dot(o_buf[rows(c), :], wo_buf[slot, :, cols], preferred_element_type=jnp.float32)
            a = acc[rows(c), cols]
            if slot == 0:
                a = jnp.where(g == 0, 0.0, a)
            t = a + y
            acc[rows(c), cols] = t
            if slot == NB - 1:
                out_buf[br, rows(c), cols] = t.astype(jnp.bfloat16)

                @pl.when(g == NG - 1)
                def _():
                    pltpu.make_async_copy(out_buf.at[br, rows(c), cols],
                                          out.at[rows(c), pl.ds(br * D + lo, hi - lo)],
                                          sems.at[_SEM_OUT + br]).start()

        def each(fn):
            return lambda c: [fn(b) for b in range(c * BPC, (c + 1) * BPC)]

        return {"Q": lambda c: q_head(c, pl.ds(0, G * DH)),
                "q": lambda i: q_head(i // G, pl.ds(i % G * DH, DH)),
                "K": each(score), "k": score, "P": each(value), "O": o_proj,
                "L": lambda c: o_proj(c, 0, OSPLIT), "R": lambda c: o_proj(c, OSPLIT, D)}

    start_slot(0, 0, 0, with_x=True)
    start_slot(1, 0, 1)

    def body(it, carry):
        br = jnp.right_shift(it, 1)
        odd = jnp.bitwise_and(it, 1)
        g0 = odd * NB

        def prefetch(j):
            jj = (j + 2) % NB
            if j < 2:
                for b_ in range(2):
                    pl.when(br == b_)(lambda b_=b_: start_slot(jj, b_, g0 + j + 2))
                return
            for nxt in range(1, NIT):
                pl.when(it == nxt - 1)(
                    lambda nxt=nxt: start_slot(jj, nxt // 2, nxt % 2 * NB + jj, with_x=(nxt == NIT // 2)))

        for j in range(NB):
            stage = stages(j, br, g0 + j)
            for t in _SCHED[j]:
                if t == "D":
                    prefetch(j)
                elif t.startswith("w:"):
                    for n in t[2:].split(","):
                        if n[0] == "x":
                            pl.when(odd == 0)(lambda n=n: copy(j, n).wait())
                        else:
                            copy(j, n).wait()
                else:
                    stage[t[0]](int(t[1:]))
        return carry

    lax.fori_loop(0, NIT, body, 0)

    for br in range(2):
        pltpu.make_async_copy(out_buf.at[br], out.at[:, pl.ds(br * D, D)], sems.at[_SEM_OUT + br]).wait()


@jax.jit
def pallas_concat_heads__mha_block_cached__mha_block_cached__near_ridge_kernel(
    A_x: jax.Array,
    A_k_cache: jax.Array,
    A_v_cache: jax.Array,
    A_wq: jax.Array,
    A_wo: jax.Array,
    B_x: jax.Array,
    B_k_cache: jax.Array,
    B_v_cache: jax.Array,
    B_wq: jax.Array,
    B_wo: jax.Array,
):
    r3 = lambda t: t.reshape(B, H * SK, DH)
    r2 = lambda t: t.reshape(M, D)
    any_spec = pl.BlockSpec(memory_space=pl.ANY)
    out = pl.pallas_call(
        _kernel,
        out_shape=jax.ShapeDtypeStruct((M, 2 * D), jnp.bfloat16),
        in_specs=[any_spec] * 10,
        out_specs=any_spec,
        scratch_shapes=[
            pltpu.VMEM((2, M, D), jnp.bfloat16),
            pltpu.VMEM((NB + 1, D, G * DH), jnp.bfloat16),
            pltpu.VMEM((NB + 1, G * DH, D), jnp.bfloat16),
            pltpu.VMEM((NB, B, G * SK, DH), jnp.bfloat16),
            pltpu.VMEM((NB, B, G * SK, DH), jnp.bfloat16),
            pltpu.VMEM((M, G * DH), jnp.bfloat16),
            pltpu.VMEM((M, G * DH), jnp.bfloat16),
            pltpu.VMEM((M, D), jnp.float32),
            pltpu.VMEM((2, M, D), jnp.bfloat16),
            pltpu.SemaphoreType.DMA((_SEM_OUT + 2,)),
        ],
        compiler_params=pltpu.CompilerParams(
            vmem_limit_bytes=64 * 1024 * 1024,
            disable_bounds_checks=True,
            disable_semaphore_checks=True,
            flags={"XLA_TPU_FORCE_LP_LLO_SCHEDULER": True, "XLA_TPU_RESCHEDULE_DMA_DONES": True},
        ),
    )(r2(A_x), r3(A_k_cache), r3(A_v_cache), A_wq, A_wo,
      r2(B_x), r3(B_k_cache), r3(B_v_cache), B_wq, B_wo)
    return out.reshape(B, SQ, 2 * D)
```

```python
import math

import jax
import jax.numpy as jnp
from jax import lax
from jax.experimental import pallas as pl
from jax.experimental.pallas import tpu as pltpu

B, SQ, D = 32, 32, 640
H, SK, DH = 32, 32, 128
M = B * SQ
SCALE_LOG2E = DH ** -0.5 * math.log2(math.e)

G = 4
NG = H // G
CH = 128
BPC = CH // SQ
NB = 4
NIT = 2 * NG // NB
XS = (0, 128, 256, 512, 896, M)
KBS = (0, 16, B)
VBS = (0, 8, 16, B)
OSPLIT = 384

_SLOT0 = "wq x0 x1 x2 x3 x4 k0 v0 v1 woL woR k1 v2 po0 po1 pq0 pq1".split()
_SLOTN = ("wq", "k", "v", "wo")
_SEM = {(0, n): i for i, n in enumerate(_SLOT0)}
_SEM.update({(j, n): len(_SLOT0) + 4 * (j - 1) + i for j in range(1, NB) for i, n in enumerate(_SLOTN)})
_SEM_OUT = len(_SEM)

_TAIL = "K2 Q4 P2 O1 K3 Q5 P3 O2 K4 Q6 P4 O3 K5 Q7 P5 K6 O4 P6 K7 O5 P7 O6"
_SCHED = (
    "w:wq,x0 Q0 w:x1 Q1 D w:x2 Q2 Q3 w:x3 Q4 Q5 Q6 w:x4 Q7 w:k0,v0 K0 K1 K2 K3 P0 P1 w:v1 P2 P3 "
    "w:woL L0 w:woR R0 O1 w:k1 K4 K5 O2 w:po0,v2 P4 P5 K6 K7 O3 P6 P7 O4 O5 O6 O7",
    "w:po1,wq Q0 Q1 D w:k K0 Q2 w:pq0,v P0 K1 Q3 P1 w:pq1,wo O0 " + _TAIL + " O7",
    "w:wq Q0 Q1 D w:k K0 Q2 w:v P0 K1 Q3 P1 w:wo O0 " + _TAIL + " O7",
    "w:wq Q0 Q1 D w:k K0 Q2 w:v P0 K1 Q3 P1 w:wo O0 " + _TAIL + " L7 R7",
)

_EXTRA_PARAMS = {}
if tuple(int(v) for v in jax.__version__.split(".")[:2]) >= (0, 12):
    _EXTRA_PARAMS = dict(
        disable_semaphore_checks=True,
        flags={"XLA_TPU_FORCE_LP_LLO_SCHEDULER": True, "XLA_TPU_RESCHEDULE_DMA_DONES": True},
    )


def _interleave(tokens):
    out, i = [], 0
    while i < len(tokens):
        j = i + 1
        while j < len(tokens) and tokens[j][0] not in "QKPOLR":
            j += 1
        if tokens[i][0] == "K" and j < len(tokens) and tokens[j][0] == "Q":
            c, d = int(tokens[i][1:]), int(tokens[j][1:])
            for u in range(2):
                out += [f"k{4 * c + 2 * u + w}" for w in range(2)] + [f"q{4 * d + 2 * u + w}" for w in range(2)]
            out += tokens[i + 1:j]
            i = j + 1
        else:
            out.append(tokens[i])
            i += 1
    return out


_SCHED = tuple(_interleave(s.split()) for s in _SCHED)


def _softmax_tile(q4, k4):
    st = lax.dot_general(k4, q4, (((1,), (1,)), ((), ())), preferred_element_type=jnp.float32)
    lg = lax.broadcasted_iota(jnp.int32, (SK, G * SQ), 1) // SQ
    c = jnp.where(lg == 0, st[0:32],
                  jnp.where(lg == 1, st[32:64], jnp.where(lg == 2, st[64:96], st[96:128])))
    e = jnp.exp2((c - jnp.max(c, axis=0, keepdims=True)) * SCALE_LOG2E)
    p = e / jnp.sum(e, axis=0, keepdims=True)
    return jnp.concatenate([jnp.where(lg == h, p, 0.0) for h in range(G)], axis=0).astype(jnp.bfloat16)


def _kernel(ax, ak, av, awq, awo, bx, bk, bv, bwq, bwo, out,
            x_buf, wq_buf, wo_buf, k_buf, v_buf, q_buf, o_buf, acc, out_buf, sems):
    srcs = ((ax, ak, av, awq, awo), (bx, bk, bv, bwq, bwo))

    def copy(j, n, br=0, g=0, x_slot=None):
        xs, xk, xv, xwq, xwo = srcs[br]
        sem = sems.at[_SEM[(0 if n[0] in "xp" else j, n)]]
        hs, gs = pl.ds(g * G * SK, G * SK), pl.ds(g * G * DH, G * DH)
        if n == "wq":
            return pltpu.make_async_copy(xwq.at[:, gs], wq_buf.at[j], sem)
        if n == "wo":
            return pltpu.make_async_copy(xwo.at[gs, :], wo_buf.at[j], sem)
        if n in ("woL", "woR"):
            cols = pl.ds(0, OSPLIT) if n == "woL" else pl.ds(OSPLIT, D - OSPLIT)
            return pltpu.make_async_copy(xwo.at[gs, cols], wo_buf.at[j, :, cols], sem)
        if n in ("k", "v"):
            src, buf = (xk, k_buf) if n == "k" else (xv, v_buf)
            return pltpu.make_async_copy(src.at[:, hs, :], buf.at[j], sem)
        if n[0] == "p":
            buf = wo_buf if n[1] == "o" else wq_buf
            return pltpu.make_async_copy(xwq.at[pl.ds(0, 16), pl.ds(0, 128)],
                                         buf.at[NB, pl.ds(16 * int(n[2]), 16), pl.ds(0, 128)], sem)
        i = int(n[1:])
        if n[0] == "x":
            r = pl.ds(XS[i], XS[i + 1] - XS[i])
            return pltpu.make_async_copy(xs.at[r], x_buf.at[br if x_slot is None else x_slot, r], sem)
        bs, src, buf = (KBS, xk, k_buf) if n[0] == "k" else (VBS, xv, v_buf)
        r = pl.ds(bs[i], bs[i + 1] - bs[i])
        return pltpu.make_async_copy(src.at[r, hs, :], buf.at[j, r], sem)

    def start_slot(j, br, g, with_x=False):
        for n in (_SLOT0 if j == 0 else _SLOTN):
            if with_x or n[0] != "x":
                copy(j, n, br, g).start()

    def rows(c):
        return pl.ds(c * CH, CH)

    def stages(slot, br, g):
        probs = {}

        def q_head(c, cols):
            q = jnp.dot(x_buf[br, rows(c), :], wq_buf[slot, :, cols], preferred_element_type=jnp.float32)
            q_buf[rows(c), cols] = q.astype(jnp.bfloat16)

        def score(b):
            r = pl.ds(b * SQ, SQ)
            q4 = jnp.concatenate([q_buf[r, h * DH:(h + 1) * DH] for h in range(G)], axis=0)
            probs[b] = _softmax_tile(q4, k_buf[slot, b])

        def value(b):
            r = pl.ds(b * SQ, SQ)
            o4 = lax.dot_general(probs.pop(b), v_buf[slot, b], (((0,), (0,)), ((), ())),
                                 preferred_element_type=jnp.float32).astype(jnp.bfloat16)
            for h in range(G):
                o_buf[r, h * DH:(h + 1) * DH] = o4[h * SQ:(h + 1) * SQ]

        def o_proj(c, lo=0, hi=D):
            cols = pl.ds(lo, hi - lo)
            y = jnp.dot(o_buf[rows(c), :], wo_buf[slot, :, cols], preferred_element_type=jnp.float32)
            a = acc[rows(c), cols]
            if slot == 0:
                a = jnp.where(g == 0, 0.0, a)
            t = a + y
            acc[rows(c), cols] = t
            if slot == NB - 1:
                out_buf[br, rows(c), cols] = t.astype(jnp.bfloat16)

                @pl.when(g == NG - 1)
                def _():
                    pltpu.make_async_copy(out_buf.at[br, rows(c), cols],
                                          out.at[rows(c), pl.ds(br * D + lo, hi - lo)],
                                          sems.at[_SEM_OUT + br]).start()

        def each(fn):
            return lambda c: [fn(b) for b in range(c * BPC, (c + 1) * BPC)]

        return {"Q": lambda c: q_head(c, pl.ds(0, G * DH)),
                "q": lambda i: q_head(i // G, pl.ds(i % G * DH, DH)),
                "K": each(score), "k": score, "P": each(value), "O": o_proj,
                "L": lambda c: o_proj(c, 0, OSPLIT), "R": lambda c: o_proj(c, OSPLIT, D)}

    start_slot(0, 0, 0, with_x=True)
    start_slot(1, 0, 1)

    def body(it, carry):
        br = jnp.right_shift(it, 1)
        odd = jnp.bitwise_and(it, 1)
        g0 = odd * NB

        def prefetch(j):
            jj = (j + 2) % NB
            if j < 2:
                for b_ in range(2):
                    pl.when(br == b_)(lambda b_=b_: start_slot(jj, b_, g0 + j + 2))
                return
            for nxt in range(1, NIT):
                pl.when(it == nxt - 1)(
                    lambda nxt=nxt: start_slot(jj, nxt // 2, nxt % 2 * NB + jj, with_x=(nxt == NIT // 2)))

        for j in range(NB):
            stage = stages(j, br, g0 + j)
            for t in _SCHED[j]:
                if t == "D":
                    prefetch(j)
                elif t.startswith("w:"):
                    for n in t[2:].split(","):
                        if n[0] == "x":
                            pl.when(odd == 0)(lambda n=n: copy(j, n, x_slot=br).wait())
                        else:
                            copy(j, n).wait()
                else:
                    stage[t[0]](int(t[1:]))
        return carry

    lax.fori_loop(0, NIT, body, 0)

    for br in range(2):
        pltpu.make_async_copy(out_buf.at[br], out.at[:, pl.ds(br * D, D)], sems.at[_SEM_OUT + br]).wait()


@jax.jit
def pallas_concat_heads__mha_block_cached__mha_block_cached__near_ridge_kernel(
    A_x: jax.Array,
    A_k_cache: jax.Array,
    A_v_cache: jax.Array,
    A_wq: jax.Array,
    A_wo: jax.Array,
    B_x: jax.Array,
    B_k_cache: jax.Array,
    B_v_cache: jax.Array,
    B_wq: jax.Array,
    B_wo: jax.Array,
):
    r3 = lambda t: t.reshape(B, H * SK, DH)
    r2 = lambda t: t.reshape(M, D)
    any_spec = pl.BlockSpec(memory_space=pl.ANY)
    out = pl.pallas_call(
        _kernel,
        out_shape=jax.ShapeDtypeStruct((M, 2 * D), jnp.bfloat16),
        in_specs=[any_spec] * 10,
        out_specs=any_spec,
        scratch_shapes=[
            pltpu.VMEM((2, M, D), jnp.bfloat16),
            pltpu.VMEM((NB + 1, D, G * DH), jnp.bfloat16),
            pltpu.VMEM((NB + 1, G * DH, D), jnp.bfloat16),
            pltpu.VMEM((NB, B, G * SK, DH), jnp.bfloat16),
            pltpu.VMEM((NB, B, G * SK, DH), jnp.bfloat16),
            pltpu.VMEM((M, G * DH), jnp.bfloat16),
            pltpu.VMEM((M, G * DH), jnp.bfloat16),
            pltpu.VMEM((M, D), jnp.float32),
            pltpu.VMEM((2, M, D), jnp.bfloat16),
            pltpu.SemaphoreType.DMA((_SEM_OUT + 2,)),
        ],
        compiler_params=pltpu.CompilerParams(
            vmem_limit_bytes=64 * 1024 * 1024,
            disable_bounds_checks=True,
            **_EXTRA_PARAMS,
        ),
    )(r2(A_x), r3(A_k_cache), r3(A_v_cache), A_wq, A_wo,
      r2(B_x), r3(B_k_cache), r3(B_v_cache), B_wq, B_wo)
    return out.reshape(B, SQ, 2 * D)
```
